```python
import os as _os
_os.environ.setdefault("JAX_PLATFORMS", "cpu")
import jax
import jax.numpy as jnp

def _softmax(x, axis=-1):
    return jax.nn.softmax(x, axis=axis)
def _gelu(x):
    return jax.nn.gelu(x, approximate=True)
def _silu(x):
    return jax.nn.silu(x)
def _sigmoid(x):
    return jax.nn.sigmoid(x)
def _layernorm(x, axis=-1, eps=1e-5):
    m = jnp.mean(x, axis=axis, keepdims=True)
    v = jnp.var(x, axis=axis, keepdims=True)
    return (x - m) / jnp.sqrt(v + eps)
def _scatter_add(tgt, idx, src, axis=0):
    return tgt.at[idx].add(src)
def _segment_sum(src, seg, n):
    return jax.ops.segment_sum(src, seg, n)
class _Rng:
    def __init__(self, key):
        self._k = key
    def _next(self):
        self._k, sub = jax.random.split(self._k)
        return sub
    def normal(self, shape):
        return jax.random.normal(self._next(), shape, dtype=jnp.bfloat16)
    def randint(self, lo, hi, shape):
        return jax.random.randint(self._next(), shape, lo, hi, dtype=jnp.int32)
    def uniform(self, shape, lo=0.0, hi=1.0):
        return jax.random.uniform(self._next(), shape, jnp.bfloat16, lo, hi)
    def permutation(self, n):
        return jax.random.permutation(self._next(), n)


kernel_name = 'concat_heads__gqa_block_cached__mha_block_cached__near_ridge'

def setup_inputs():
    _rng = _Rng(jax.random.key(int.from_bytes(__import__("os").urandom(4), "little")))
    _w = (lambda a: (lambda t: t.astype(jnp.bfloat16) if jnp.issubdtype(t.dtype, jnp.floating) else t)(jnp.asarray(a)))
    def _A_setup():
        B, Sq, D = 8, 96, 640
        Hq, Hkv, Sk, Dh = 32, 32, 512, 128
        assert Hq % Hkv == 0, (Hq, Hkv)
        return {
            "x": _w((lambda *s: _rng.normal(s) * 0.8)(B, Sq, D)),
            "k_cache": _w((lambda *s: _rng.normal(s) * 0.8)(B, Hkv, Sk, Dh)),
            "v_cache": _w((lambda *s: _rng.normal(s) * 0.05)(B, Hkv, Sk, Dh)),
            "wq": _w((lambda *s: _rng.normal(s) * 0.8)(D, Hq * Dh) * (D ** -0.5)),
            "wo": _w((lambda *s: _rng.normal(s) * 0.05)(Hq * Dh, D) * ((Hq * Dh) ** -0.5)),
        }
    _A_in = _A_setup()

    def _B_setup():
        B, Sq, D = 8, 96, 640
        H, Sk, Dh = 32, 512, 128
        return {
            "x": _w((lambda *s: _rng.normal(s) * 0.8)(B, Sq, D)),
            "k_cache": _w((lambda *s: _rng.normal(s) * 0.8)(B, H, Sk, Dh)),
            "v_cache": _w((lambda *s: _rng.normal(s) * 0.05)(B, H, Sk, Dh)),
            "wq": _w((lambda *s: _rng.normal(s) * 0.8)(D, H * Dh) * (D ** -0.5)),
            "wo": _w((lambda *s: _rng.normal(s) * 0.05)(H * Dh, D) * ((H * Dh) ** -0.5)),
        }
    _B_in = _B_setup()

    return {
        "A_x": _A_in["x"],
        "A_k_cache": _A_in["k_cache"],
        "A_v_cache": _A_in["v_cache"],
        "A_wq": _A_in["wq"],
        "A_wo": _A_in["wo"],
        "B_x": _B_in["x"],
        "B_k_cache": _B_in["k_cache"],
        "B_v_cache": _B_in["v_cache"],
        "B_wq": _B_in["wq"],
        "B_wo": _B_in["wo"],
    }

def reference(A_x, A_k_cache, A_v_cache, A_wq, A_wo, B_x, B_k_cache, B_v_cache, B_wq, B_wo):
    def _A_ref(x, k_cache, v_cache, wq, wo):
        B, Sq, D = x.shape
        Hq, Dh = 32, 128
        Hkv = k_cache.shape[1]
        rep = Hq // Hkv
        q = (lambda x, *d: x.transpose(*d))((x @ wq).reshape(B, Sq, Hq, Dh), 0, 2, 1, 3)
        k = jnp.repeat(k_cache, rep, axis=1)
        v = jnp.repeat(v_cache, rep, axis=1)
        scores = jnp.einsum("bhqd,bhkd->bhqk", q, k) * (Dh ** -0.5)
        p = _softmax(scores, axis=-1)
        o = jnp.einsum("bhqk,bhkd->bhqd", p, v)
        return (lambda x, *d: x.transpose(*d))(o, 0, 2, 1, 3).reshape(B, Sq, Hq * Dh) @ wo

    def _B_ref(x, k_cache, v_cache, wq, wo):
        B, Sq, D = x.shape
        H, Dh = 32, 128
        q = (lambda x, *d: x.transpose(*d))((x @ wq).reshape(B, Sq, H, Dh), 0, 2, 1, 3)
        scores = jnp.einsum("bhqd,bhkd->bhqk", q, k_cache) * (Dh ** -0.5)
        p = _softmax(scores, axis=-1)
        o = jnp.einsum("bhqk,bhkd->bhqd", p, v_cache)
        return (lambda x, *d: x.transpose(*d))(o, 0, 2, 1, 3).reshape(B, Sq, H * Dh) @ wo

    a = _A_ref(A_x, A_k_cache, A_v_cache, A_wq, A_wo)
    b = _B_ref(B_x, B_k_cache, B_v_cache, B_wq, B_wo)
    return jnp.concatenate([a, b], axis=-1)
```

```python
import math
import jax, jax.numpy as jnp
from jax import lax
from jax.experimental import pallas as pl
from jax.experimental.pallas import tpu as pltpu

B, Sq, D, H, Sk, Dh = 8, 96, 640, 32, 512, 128
M = B * Sq
C = (Dh ** -0.5) * math.log2(math.e)
NT = (((1,), (1,)), ((), ()))
f32, bf16 = jnp.float32, jnp.bfloat16

def make(LA=11, Gq=2, dma=True, compute=True, order='SQPO', flags=None, dP=1, dO=2, po='r0 b2 b1 a r1', XR=16, OR=32, wpos=0, aw=3, na=4,
         ipos=2, shrink=(), nbc=True, nsc=False, wr_out=True, NSEM=4, orders=None, wj=None, opos=None):
    U, G, R, NS = 4, 2, 128, 8
    NP = H * G; N = 2 * NP
    WL = Gq * G
    QR, WR = D // WL, Dh // G
    pieces = []
    for j in range(32):
        bt = {nm: (j >> i) & 1 for i, nm in enumerate(po.split())}
        pieces.append((bt['a'], bt['b1'] + 2 * bt['b2'], bt['r0'] + 2 * bt['r1']))
    if shrink: assert 'a' in po.split()[:3]
    st_ = lambda a: isinstance(a, int)
    dv = lambda a, k: a // k if st_(a) else lax.shift_right_logical(a, k.bit_length() - 1)
    md = lambda a, k: a % k if st_(a) else a & (k - 1)
    mo = lambda v, k: v if st_(v) else pl.multiple_of(v, k)
    def kern(ax, ak, av, awq, awo, bx, bk, bv, bwq, bwo, out, xb, wqb, wob, kb, vb, qb, pb, lb, ob, acc, res, sem, osem):
        srcs = [(ak, av, awq, awo), (bk, bv, bwq, bwo)]
        def w_regions(m):
            return mo(md(m, WL) * QR, 8), pl.ds(mo(dv(m, WL) * (Gq * Dh), Gq * Dh), Gq * Dh), mo(m * WR, WR)
        def w_copies(p, m, s):
            q0, qc, o0 = w_regions(m)
            cq = [(srcs[p][2].at[pl.ds(q0 + i * (QR // 2), QR // 2), qc], wqb.at[p, pl.ds(q0 + i * (QR // 2), QR // 2), qc], s) for i in range(2)]
            co = [(srcs[p][3].at[pl.ds(o0 + i * (WR // 2), WR // 2)], wob.at[p, pl.ds(o0 + i * (WR // 2), WR // 2)], s) for i in range(2)]
            return [cq[0], co[0], co[1], cq[1]]
        def kv_copies(p, m, part):
            h, g, slot, s = dv(m, G), md(m, G), md(m, NS), sem.at[md(m, NSEM)]
            cs = []
            for i in range(8):
                if st_(part): a, b, r = pieces[8 * part + i]
                else:
                    a, b, r = pieces[i]
                    for bit in range(2):
                        _, db, dr = pieces[8 << bit]
                        x = md(dv(part, 1 << bit), 2)
                        b, r = b + db * x if db else b, r + dr * x if dr else r
                rr = pl.ds(mo(r * R, R), R)
                cs.append((srcs[p][a].at[b * G + g, h, rr], (kb, vb)[a].at[slot, b, rr], s))
            return cs
        def start(cs):
            for j, c in enumerate(cs): pltpu.make_async_copy(*c).start(priority=j % 2)
        def out_copies(p, row, nrows):
            return [(res.at[p, pl.ds(row + r, OR)], out.at[pl.ds(row + r, OR), pl.ds(p * D, D)], osem.at[0]) for r in range(0, nrows, OR)]
        def prefetch(n, j):
            m, part = n + (j + LA) // U, (j + LA) % U
            for p in range(2):
                if p == 1 and shrink:
                    F = n * U + j
                    f = F + LA - sum((F > N * U - s).astype(jnp.int32) for s in shrink)
                    ok = (f >= NP * U) & (f < N * U)
                    for s in shrink:
                        if (-s) % U == j: ok = ok & (F != N * U - s)
                    pl.when(ok)(lambda: start(kv_copies(1, dv(f, U) - NP, md(f, U))))
                else:
                    pl.when((m >= p * NP) & (m < (p + 1) * NP))(lambda: start(kv_copies(p, m - p * NP, part)))
                if part == wpos:
                    pl.when((m + WL >= p * NP) & (m + WL < (p + 1) * NP))(lambda: start(w_copies(p, m + WL - p * NP, sem.at[md(m, NSEM)])))
        def write_a(n, j):
            for i in range(na):
                F = N * U - LA + aw + i
                assert F < N * U
                if F % U == j: pl.when(n == F // U)(lambda: start(out_copies(0, M // na * i, M // na)))
        def wait(n):
            slot, s = md(n, NS), sem.at[md(n, NSEM)]
            for buf in (kb, vb): pltpu.make_async_copy(buf.at[slot], buf.at[slot], s).wait()
            @pl.when(n + WL < N)
            def _():
                m = n + WL
                q0, qc, o0 = w_regions(md(m, NP))
                for r in (wqb.at[dv(m, NP), pl.ds(q0, QR), qc], wob.at[dv(m, NP), pl.ds(o0, WR)]): pltpu.make_async_copy(r, r, s).wait()
        xc = [(x.at[pl.ds(r, XR)], xb.at[p, pl.ds(r, XR)], osem.at[0]) for r in range(0, M, XR) for p, x in enumerate((ax, bx))]
        xc += [c for m in range(WL) for c in w_copies(0, m, osem.at[0])]
        if dma: start(xc)
        acc[...] = jnp.zeros_like(acc)
        for r in (pb, lb, ob): r[...] = jnp.zeros_like(r)
        for b in range(U - dP, U): vb[NS - 1, b] = jnp.zeros((Sk, Dh), bf16)
        if dma:
            for f in range(LA):
                start(kv_copies(0, f // U, f % U) + (w_copies(0, f // U + WL, sem.at[f // U]) if f % U == wpos else []))
            for c in xc: pltpu.make_async_copy(*c).wait()
        def softmax(s):
            e = jnp.exp2(s - jnp.max(s, axis=-1, keepdims=True))
            return e.astype(bf16), jnp.broadcast_to(1.0 / jnp.sum(e, axis=-1, keepdims=True), (Sq, Dh))
        def where(n, u):
            m = n + u // U
            slot = md(m + NS, NS)
            if not st_(m) and u < 0: m = jnp.maximum(m, 0)
            if not st_(m) and u >= U: m = jnp.minimum(m, N - 1)
            return slot, dv(m, NP), pl.ds(mo(dv(md(m, NP), G) * Dh, Dh), Dh), mo(((u % U) * G + md(m, G)) * Sq, Sq)
        def qproj(n, u):
            _, p, hd, row = where(n, u)
            return (jnp.dot(xb[p, pl.ds(row, Sq), :], wqb[p, :, hd], preferred_element_type=f32) * C).astype(bf16)
        def steps(n, js, drain):
            q, e, o = {}, {}, {}
            for j in js:
                od = orders[j] if (orders and not drain) else order
                for si, st in enumerate(od):
                    if dma and not drain and si == (ipos[j] if isinstance(ipos, tuple) else ipos): prefetch(n, j)
                    if dma and wr_out and not drain and si == (opos if opos is not None else (ipos[j] if isinstance(ipos, tuple) else ipos)): write_a(n, j)
                    u = j - dict(Q=-1, S=0, P=dP, O=dO)[st]
                    if (drain and u >= 0) or not compute: continue
                    slot, p, hd, row = where(n, u)
                    if st == 'Q':
                        if u < U: q[u] = qproj(n, u)
                        else: qb[...] = qproj(n, u)
                    if st == 'S':
                        s = lax.dot_general(q[u] if u in q else qb[...], kb[slot, u % U], NT, preferred_element_type=f32)
                        if u + dP < U: e[u] = softmax(s)
                        else: pb[u + dP - U], lb[u + dP - U] = softmax(s)
                    if st == 'P':
                        ee, r = e[u] if u in e else (pb[u + dP], lb[u + dP])
                        v = (jnp.dot(ee, vb[slot, u % U], preferred_element_type=f32) * r).astype(bf16)
                        if u + dO < U or drain: o[u] = v
                        else: ob[u + dO - U] = v
                    if st == 'O':
                        rows = pl.ds(row, Sq)
                        a = acc[p, rows, :] + jnp.dot(o[u] if u in o else ob[u + dO], wob[p, hd, :], preferred_element_type=f32)
                        if not drain: acc[p, rows, :] = a
                        res[p, rows, :] = a.astype(bf16)
                        if dma and wr_out:
                            if drain: start(out_copies(1, row, Sq))
                            else: pl.when(n + u // U >= N - G)(lambda: start(out_copies(1, row, Sq)))
        qb[...] = qproj(0, 0)
        def body(n, c):
            if dma: wait(n)
            steps(n, range(U), False)
            return c
        lax.fori_loop(0, N, body, 0)
        steps(N, range(dO), True)
        if dma and wr_out:
            for p in range(2 if compute else 1):
                for c in out_copies(p, 0, M): pltpu.make_async_copy(*c).wait()
    def f(ax, ak, av, awq, awo, bx, bk, bv, bwq, bwo):
        V = pltpu.VMEM
        o = pl.pallas_call(kern, out_shape=jax.ShapeDtypeStruct((M, 2 * D), bf16),
            in_specs=[pl.BlockSpec(memory_space=pltpu.HBM)] * 10, out_specs=pl.BlockSpec(memory_space=pltpu.HBM),
            scratch_shapes=[V((2, M, D), bf16), V((2, D, H * Dh), bf16), V((2, H * Dh, D), bf16), V((NS, U, Sk, Dh), bf16), V((NS, U, Sk, Dh), bf16),
                V((Sq, Dh), bf16), V((dP, Sq, Sk), bf16), V((dP, Sq, Dh), f32), V((dO - dP, Sq, Dh), bf16), V((2, M, D), f32), V((2, M, D), bf16),
                pltpu.SemaphoreType.DMA((NSEM,)), pltpu.SemaphoreType.DMA((1,))],
            compiler_params=pltpu.CompilerParams(vmem_limit_bytes=64 * 2**20, disable_bounds_checks=nbc, disable_semaphore_checks=nsc, flags=flags),
        )(ax.reshape(M, D), ak, av, awq, awo, bx.reshape(M, D), bk, bv, bwq, bwo)
        return o.reshape(B, Sq, 2 * D)
    return jax.jit(f)


_impl = make(ipos=0)


@jax.jit
def pallas_concat_heads__gqa_block_cached__mha_block_cached__near_ridge_kernel(
        A_x, A_k_cache, A_v_cache, A_wq, A_wo, B_x, B_k_cache, B_v_cache, B_wq, B_wo):
    return _impl(A_x, A_k_cache, A_v_cache, A_wq, A_wo, B_x, B_k_cache, B_v_cache, B_wq, B_wo)
```

```python
import math

import jax
import jax.numpy as jnp
from jax import lax
import jax.experimental.pallas as pl
import jax.experimental.pallas.tpu as pltpu

B, SQ, D, H, SK, DH = 8, 96, 640, 32, 512, 128
M = B * SQ
QK_SCALE = (DH ** -0.5) * math.log2(math.e)

UNITS = 4
GROUPS_PER_HEAD = B // UNITS
GROUPS_PER_PROBLEM = H * GROUPS_PER_HEAD
GROUPS = 2 * GROUPS_PER_PROBLEM

KV_SLOTS = 8
SEM_SLOTS = 4
LOOKAHEAD = (2, 3)
KV_ROWS = 128
X_ROWS = 16
OUT_ROWS = 32

WQ_HEADS = 2
W_AHEAD = WQ_HEADS * GROUPS_PER_HEAD
WQ_ROWS = D // W_AHEAD
WO_ROWS = DH // GROUPS_PER_HEAD

A_WRITE_START = 7
A_WRITE_SLOTS = 4

SEM_K, SEM_V, SEM_WQ, SEM_WO = range(4)


def _div(a, k):
    return a // k if isinstance(a, int) else lax.shift_right_logical(a, k.bit_length() - 1)


def _mod(a, k):
    return a % k if isinstance(a, int) else a & (k - 1)


def _aligned(a, k):
    return a if isinstance(a, int) else pl.multiple_of(a, k)


def _kernel(ax, ak, av, awq, awo, bx, bk, bv, bwq, bwo, out,
            x_buf, wq_buf, wo_buf, k_buf, v_buf,
            q_carry, e_carry, r_carry, o_carry, acc, res, sems, io_sem):
    caches = ((ak, av), (bk, bv))
    weights = ((awq, awo), (bwq, bwo))

    def kv_piece(p, m, part, i):
        is_v = part % 2
        unit = 2 * ((i >> 1) & 1) + (i >> 2)
        rows = pl.ds((2 * (part // 2) + i % 2) * KV_ROWS, KV_ROWS)
        batch = unit * GROUPS_PER_HEAD + _mod(m, GROUPS_PER_HEAD)
        return (caches[p][is_v].at[batch, _div(m, GROUPS_PER_HEAD), rows],
                (k_buf, v_buf)[is_v].at[_mod(m, KV_SLOTS), unit, rows],
                sems.at[(SEM_K, SEM_V)[is_v], _mod(m, SEM_SLOTS)])

    def weight_chunk(c):
        cols = pl.ds(_aligned(_div(c, W_AHEAD) * (WQ_HEADS * DH), WQ_HEADS * DH), WQ_HEADS * DH)
        return _aligned(_mod(c, W_AHEAD) * WQ_ROWS, 8), cols, _aligned(c * WO_ROWS, WO_ROWS)

    def weight_piece(p, c, i, sem=None):
        wq_row, wq_cols, wo_row = weight_chunk(c)
        slot = _mod(c, SEM_SLOTS)
        if i in (0, 3):
            rows = pl.ds(wq_row + (i // 2) * (WQ_ROWS // 2), WQ_ROWS // 2)
            return (weights[p][0].at[rows, wq_cols], wq_buf.at[p, rows, wq_cols],
                    sems.at[SEM_WQ, slot] if sem is None else sem)
        rows = pl.ds(wo_row + (i // 2) * (WO_ROWS // 2), WO_ROWS // 2)
        return (weights[p][1].at[rows], wo_buf.at[p, rows],
                sems.at[SEM_WO, slot] if sem is None else sem)

    def out_piece(p, row):
        rows = pl.ds(row, OUT_ROWS)
        return res.at[p, rows], out.at[rows, pl.ds(p * D, D)], io_sem.at[0]

    def start(pieces):
        for i, piece in enumerate(pieces):
            pltpu.make_async_copy(*piece).start(priority=i % 2)

    def start_if_in_range(index, piece_fn, priority):
        for p in range(2):
            first = p * GROUPS_PER_PROBLEM

            @pl.when((index >= first) & (index < first + GROUPS_PER_PROBLEM))
            def _():
                pltpu.make_async_copy(*piece_fn(p, index - first)).start(priority=priority)

    def prefetch(n, part):
        for i in range(8):
            start_if_in_range(n + LOOKAHEAD[i % 2],
                              lambda p, m: kv_piece(p, m, part, i), i % 2)
        if part == 0:
            for i in range(4):
                start_if_in_range(n + LOOKAHEAD[i % 2] + W_AHEAD,
                                  lambda p, c: weight_piece(p, c, i), i % 2)

    def wait_group(n):
        def wait_filled(region, kind):
            pltpu.make_async_copy(region, region, sems.at[kind, _mod(n, SEM_SLOTS)]).wait()

        wait_filled(k_buf.at[_mod(n, KV_SLOTS)], SEM_K)
        wait_filled(v_buf.at[_mod(n, KV_SLOTS)], SEM_V)

        @pl.when(n + W_AHEAD < GROUPS)
        def _():
            p = _div(n + W_AHEAD, GROUPS_PER_PROBLEM)
            wq_row, wq_cols, wo_row = weight_chunk(_mod(n + W_AHEAD, GROUPS_PER_PROBLEM))
            wait_filled(wq_buf.at[p, pl.ds(wq_row, WQ_ROWS), wq_cols], SEM_WQ)
            wait_filled(wo_buf.at[p, pl.ds(wo_row, WO_ROWS)], SEM_WO)

    def write_first_output(n, j):
        rows = [b * SQ + r for r in range(0, SQ, OUT_ROWS) for b in range(B)]
        per_slot = len(rows) // A_WRITE_SLOTS
        for i in range(A_WRITE_SLOTS):
            slot = GROUPS * UNITS - A_WRITE_START + i
            if slot % UNITS == j:
                @pl.when(n == slot // UNITS)
                def _():
                    start([out_piece(0, r) for r in rows[i * per_slot:(i + 1) * per_slot]])

    def locate(n, u):
        m = n + u // UNITS
        slot = _mod(m + KV_SLOTS, KV_SLOTS)
        if not isinstance(m, int):
            if u < 0:
                m = jnp.maximum(m, 0)
            if u >= UNITS:
                m = jnp.minimum(m, GROUPS - 1)
        head = _div(_mod(m, GROUPS_PER_PROBLEM), GROUPS_PER_HEAD)
        batch = (u % UNITS) * GROUPS_PER_HEAD + _mod(m, GROUPS_PER_HEAD)
        return (slot, _div(m, GROUPS_PER_PROBLEM),
                pl.ds(_aligned(head * DH, DH), DH), _aligned(batch * SQ, SQ))

    def q_stage(n, u):
        _, p, head, row = locate(n, u)
        q = jnp.dot(x_buf[p, pl.ds(row, SQ), :], wq_buf[p, :, head],
                    preferred_element_type=jnp.float32)
        return (q * QK_SCALE).astype(jnp.bfloat16)

    def s_stage(n, u, q):
        s = lax.dot_general(q, k_buf[locate(n, u)[0], u % UNITS], (((1,), (1,)), ((), ())),
                            preferred_element_type=jnp.float32)
        e = jnp.exp2(s - jnp.max(s, axis=-1, keepdims=True))
        r = 1.0 / jnp.sum(e, axis=-1, keepdims=True)
        return e.astype(jnp.bfloat16), jnp.broadcast_to(r, (SQ, DH))

    def p_stage(n, u, e, r):
        o = jnp.dot(e, v_buf[locate(n, u)[0], u % UNITS], preferred_element_type=jnp.float32)
        return (o * r).astype(jnp.bfloat16)

    def o_stage(n, u, o):
        _, p, head, row = locate(n, u)
        rows = pl.ds(row, SQ)
        total = acc[p, rows, :] + jnp.dot(o, wo_buf[p, head, :],
                                          preferred_element_type=jnp.float32)
        res[p, rows, :] = total.astype(jnp.bfloat16)

        def write_rows():
            start([out_piece(1, row + r) for r in range(0, SQ, OUT_ROWS)])

        if isinstance(n, int):
            write_rows()
        else:
            acc[p, rows, :] = total
            pl.when(n + u // UNITS >= GROUPS - GROUPS_PER_HEAD)(write_rows)

    def group(n, carry):
        wait_group(n)
        q, er, o = q_carry[...], None, None
        for j in range(UNITS):
            er_new = s_stage(n, j, q)
            q = q_stage(n, j + 1)
            prefetch(n, j)
            write_first_output(n, j)
            o_new = p_stage(n, j - 1, *(er if j else (e_carry[...], r_carry[...])))
            o_stage(n, j - 2, o if j else o_carry[...])
            er, o = er_new, o_new
        q_carry[...] = q
        e_carry[...], r_carry[...] = er
        o_carry[...] = o
        return carry

    setup = [(x.at[pl.ds(r, X_ROWS)], x_buf.at[p, pl.ds(r, X_ROWS)], io_sem.at[0])
             for r in range(0, M, X_ROWS) for p, x in enumerate((ax, bx))]
    setup += [weight_piece(0, c, i, io_sem.at[0]) for c in range(W_AHEAD) for i in range(4)]
    queues = []
    for priority, ahead in enumerate(LOOKAHEAD):
        queue = []
        for m in range(ahead):
            for part in range(UNITS):
                queue += [kv_piece(0, m, part, i) for i in range(priority, 8, 2)]
                if part == 0:
                    queue += [weight_piece(0, m + W_AHEAD, i) for i in range(priority, 4, 2)]
        queues.append(queue)
    shared = len(setup) + len(queues[0]) - len(queues[1])
    queues = [setup[:shared:2] + setup[shared:] + queues[0], setup[1:shared:2] + queues[1]]
    pieces = [piece for pair in zip(*queues, strict=True) for piece in pair]

    start(pieces[:64])
    acc[...] = jnp.zeros_like(acc)
    for ref in (e_carry, r_carry, o_carry):
        ref[...] = jnp.zeros_like(ref)
    v_buf[KV_SLOTS - 1, UNITS - 1] = jnp.zeros((SK, DH), jnp.bfloat16)
    start(pieces[64:])
    for piece in setup:
        pltpu.make_async_copy(*piece).wait()
    q_carry[...] = q_stage(0, 0)

    lax.fori_loop(0, GROUPS, group, 0)

    o_last = p_stage(GROUPS, -1, e_carry[...], r_carry[...])
    o_stage(GROUPS, -2, o_carry[...])
    o_stage(GROUPS, -1, o_last)
    for p in range(2):
        for row in range(0, M, OUT_ROWS):
            pltpu.make_async_copy(*out_piece(p, row)).wait()


@jax.jit
def pallas_concat_heads__gqa_block_cached__mha_block_cached__near_ridge_kernel(
    A_x: jax.Array,
    A_k_cache: jax.Array,
    A_v_cache: jax.Array,
    A_wq: jax.Array,
    A_wo: jax.Array,
    B_x: jax.Array,
    B_k_cache: jax.Array,
    B_v_cache: jax.Array,
    B_wq: jax.Array,
    B_wo: jax.Array,
):
    assert A_x.shape == B_x.shape == (B, SQ, D)
    assert A_k_cache.shape == A_v_cache.shape == (B, H, SK, DH)
    assert B_k_cache.shape == B_v_cache.shape == (B, H, SK, DH)
    assert W_AHEAD % SEM_SLOTS == 0 and GROUPS_PER_PROBLEM % KV_SLOTS == 0

    hbm = pl.BlockSpec(memory_space=pltpu.HBM)
    bf16, f32 = jnp.bfloat16, jnp.float32
    out = pl.pallas_call(
        _kernel,
        out_shape=jax.ShapeDtypeStruct((M, 2 * D), bf16),
        in_specs=[hbm] * 10,
        out_specs=hbm,
        scratch_shapes=[
            pltpu.VMEM((2, M, D), bf16),
            pltpu.VMEM((2, D, H * DH), bf16),
            pltpu.VMEM((2, H * DH, D), bf16),
            pltpu.VMEM((KV_SLOTS, UNITS, SK, DH), bf16),
            pltpu.VMEM((KV_SLOTS, UNITS, SK, DH), bf16),
            pltpu.VMEM((SQ, DH), bf16),
            pltpu.VMEM((SQ, SK), bf16),
            pltpu.VMEM((SQ, DH), f32),
            pltpu.VMEM((SQ, DH), bf16),
            pltpu.VMEM((2, M, D), f32),
            pltpu.VMEM((2, M, D), bf16),
            pltpu.SemaphoreType.DMA((4, SEM_SLOTS)),
            pltpu.SemaphoreType.DMA((1,)),
        ],
        compiler_params=pltpu.CompilerParams(
            vmem_limit_bytes=64 * 1024 * 1024,
            disable_bounds_checks=True,
            disable_semaphore_checks=True,
        ),
    )(A_x.reshape(M, D), A_k_cache, A_v_cache, A_wq, A_wo,
      B_x.reshape(M, D), B_k_cache, B_v_cache, B_wq, B_wo)
    return out.reshape(B, SQ, 2 * D)
```
